```python
import os as _os
_os.environ.setdefault("JAX_PLATFORMS", "cpu")
import jax
import jax.numpy as jnp

def _softmax(x, axis=-1):
    return jax.nn.softmax(x, axis=axis)
def _gelu(x):
    return jax.nn.gelu(x, approximate=True)
def _silu(x):
    return jax.nn.silu(x)
def _sigmoid(x):
    return jax.nn.sigmoid(x)
def _layernorm(x, axis=-1, eps=1e-5):
    m = jnp.mean(x, axis=axis, keepdims=True)
    v = jnp.var(x, axis=axis, keepdims=True)
    return (x - m) / jnp.sqrt(v + eps)
def _scatter_add(tgt, idx, src, axis=0):
    return tgt.at[idx].add(src)
def _segment_sum(src, seg, n):
    return jax.ops.segment_sum(src, seg, n)
class _Rng:
    def __init__(self, key):
        self._k = key
    def _next(self):
        self._k, sub = jax.random.split(self._k)
        return sub
    def normal(self, shape):
        return jax.random.normal(self._next(), shape, dtype=jnp.bfloat16)
    def randint(self, lo, hi, shape):
        return jax.random.randint(self._next(), shape, lo, hi, dtype=jnp.int32)
    def uniform(self, shape, lo=0.0, hi=1.0):
        return jax.random.uniform(self._next(), shape, jnp.bfloat16, lo, hi)
    def permutation(self, n):
        return jax.random.permutation(self._next(), n)


kernel_name = 'gated_mix__linear_attn_block__mixer_token_mlp__prompt'

def setup_inputs():
    _rng = _Rng(jax.random.key(int.from_bytes(__import__("os").urandom(4), "little")))
    _w = (lambda a: (lambda t: t.astype(jnp.bfloat16) if jnp.issubdtype(t.dtype, jnp.floating) else t)(jnp.asarray(a)))
    def _A_setup():
        B, S, D = 1, 2048, 512
        return {
            "x": _w((lambda *s: _rng.normal(s) * 0.05)(B, S, D)),
            "wqkv": _w((lambda *s: _rng.normal(s) * 0.8)(D, 3 * D)),
            "wo": _w((lambda *s: _rng.normal(s) * 0.05)(D, D)),
        }
    _A_in = _A_setup()

    def _B_setup():
        B, S, D, F = 1, 2048, 512, 1792
        return {
            "x": _w((lambda *s: _rng.normal(s) * 0.05)(B, S, D)),
            "w1": _w((lambda *s: _rng.normal(s) * 0.1)(S, F) * (S ** -0.5)),
            "b1": _w((lambda *s: _rng.normal(s) * 0.1)(F) * 0.02),
            "w2": _w((lambda *s: _rng.normal(s) * 0.1)(F, S) * (F ** -0.5)),
            "b2": _w((lambda *s: _rng.normal(s) * 0.1)(S) * 0.02),
        }
    _B_in = _B_setup()

    return {
        "A_x": _A_in["x"],
        "A_wqkv": _A_in["wqkv"],
        "A_wo": _A_in["wo"],
        "B_x": _B_in["x"],
        "B_w1": _B_in["w1"],
        "B_b1": _B_in["b1"],
        "B_w2": _B_in["w2"],
        "B_b2": _B_in["b2"],
        "gate_w": _w((lambda *s: _rng.normal(s) * 0.05)(512) * 16.0),
    }

def reference(A_x, A_wqkv, A_wo, B_x, B_w1, B_b1, B_w2, B_b2, gate_w):
    def _A_ref(x, wqkv, wo):
        B, S, D = x.shape
        H = 32; Dh = D // H
        qkv = (lambda x, *d: x.transpose(*d))((x @ wqkv).reshape(B, S, 3, H, Dh), 2, 0, 3, 1, 4)
        q, k, v = qkv[0], qkv[1], qkv[2]
        phi = lambda t: jnp.where(t > 0, t + 1, jnp.exp(t)) + 1e-6
        pq, pk = phi(q), phi(k)
        kv = jnp.einsum("bhsd,bhse->bhde", pk, v)
        z = jnp.einsum("bhsd->bhd", pk)
        num = jnp.einsum("bhqd,bhde->bhqe", pq, kv)
        den = jnp.einsum("bhqd,bhd->bhq", pq, z)[..., None] + 1e-6
        o = num / den
        return (lambda x, *d: x.transpose(*d))(o, 0, 2, 1, 3).reshape(B, S, D) @ wo

    def _B_ref(x, w1, b1, w2, b2):
        B, S, D = x.shape
        h = _layernorm(x, axis=-1)
        u = jnp.einsum("bsd,sf->bdf", h, w1) + b1
        u = _gelu(u)
        y = jnp.einsum("bdf,fs->bds", u, w2) + b2
        return (lambda x, *d: x.transpose(*d))(y, 0, 2, 1)

    x = A_x
    g = _sigmoid((x * gate_w).sum(-1, keepdims=True))
    a = _A_ref(x, A_wqkv, A_wo)
    b = _B_ref(x, B_w1, B_b1, B_w2, B_b2)
    return g * a + (1 - g) * b
```

```python
import numpy as np
import jax
import jax.numpy as jnp
from jax import lax
import jax.experimental.pallas as pl
import jax.experimental.pallas.tpu as pltpu

S, D, F, H, DH = 2048, 512, 1792, 32, 16
BF, F32, U32 = jnp.bfloat16, jnp.float32, jnp.uint32
NT = (((1,), (1,)), ((), ()))

def _phi(t):
    return jnp.where(t > 0, t + 1.0, jnp.exp(t)) + 1e-6

def _gelu(u):
    c = float(np.sqrt(2.0 / np.pi))
    return 0.5 * u * (1.0 + jnp.tanh(c * (u + 0.044715 * (u * u * u))))

N2 = 2
FC = 128
OC = 256
N3 = 4
RP = 512
PH = 1
XMODE = 1

def ld(ref, r0, nr, cs):
    return pltpu.bitcast(ref[pl.ds(r0 // 2, nr // 2), cs], BF)
def st(ref, r0, nr, cs, val):
    ref[pl.ds(r0 // 2, nr // 2), cs] = pltpu.bitcast(val.astype(BF), U32)
def colsum8(v):
    return jnp.sum(v.reshape(v.shape[0] // 8, 8, 128), axis=0)

def kernel(x_hbm, wqkv_hbm, wo_hbm, w1_hbm, b1_hbm, w2_hbm, b2_hbm, gw_hbm, o_hbm,
           x_ref, wqkv_ref, wo_ref, w1_ref, b1_ref, w2_ref, b2_ref, gw_ref, o_ref,
           wqkvT, woT, xT_s, hT, pq, pk, vT, gu, MT, g_s, b1_s, b2_s, zb_s, gwb_s, oT_s, kv_s, sm, sems):
    XC = 512
    nx = S // XC
    xh, wqh, woh, w1h, w2h, oh = (r.bitcast(U32) for r in (x_hbm, wqkv_hbm, wo_hbm, w1_hbm, w2_hbm, o_hbm))
    cx = [pltpu.make_async_copy(xh.at[c*XC//2:(c+1)*XC//2, :], x_ref.at[c*XC//2:(c+1)*XC//2, :], sems.at[c]) for c in range(nx)]
    cw = [pltpu.make_async_copy(wqh.at[:, j*D:(j+1)*D], wqkv_ref.at[:, j*D:(j+1)*D], sems.at[4+j]) for j in range(3)]
    cgw = pltpu.make_async_copy(gw_hbm, gw_ref, sems.at[7])
    cwo = pltpu.make_async_copy(woh, wo_ref, sems.at[8])
    cb1 = pltpu.make_async_copy(b1_hbm, b1_ref, sems.at[9])
    cb2 = pltpu.make_async_copy(b2_hbm, b2_ref, sems.at[10])
    cw1 = pltpu.make_async_copy(w1h, w1_ref, sems.at[11])
    cw2 = pltpu.make_async_copy(w2h, w2_ref, sems.at[12])

    cx[0].start(); cw[0].start(); cgw.start(); cw[1].start(); cw[2].start()
    for c in range(1, nx): cx[c].start()
    cwo.start(); cb1.start(); cb2.start(); cw1.start(); cw2.start()

    for b in range(4): sm[b] = b * 128
    for b in range(3): sm[4 + b] = b * 256
    T = lambda b: slice(b*128, (b+1)*128)
    def W(j):
        st(wqkvT, j*128, 128, slice(None), ld(wqkv_ref, 0, D, T(j)).T)
    def WO(j):
        st(woT, j*128, 128, slice(None), ld(wo_ref, 0, D, T(j)).T)
    def X(b):
        s8 = None; g8 = None
        for c in range(4):
            xb = ld(x_ref, b*128, 128, T(c))
            xf = xb.astype(F32).T if XMODE == 0 else xb.T.astype(F32)
            st(xT_s, c*128, 128, T(b), xf)
            ps = colsum8(xf); pg = colsum8(xf * gwb_s[T(c), :])
            s8 = ps if s8 is None else s8 + ps
            g8 = pg if g8 is None else g8 + pg
        g_s[0:1, T(b)] = jax.nn.sigmoid(jnp.sum(g8, axis=0, keepdims=True))
        g_s[1:2, T(b)] = jnp.sum(s8, axis=0, keepdims=True) * (1.0 / D)
    def L(b):
        mean = g_s[1:2, T(b)]
        v8 = None
        for r0 in range(0, D, RP):
            xc = ld(xT_s, r0, RP, T(b)).astype(F32) - mean
            p = colsum8(xc * xc)
            v8 = p if v8 is None else v8 + p
        rstd = lax.rsqrt(jnp.sum(v8, axis=0, keepdims=True) * (1.0 / D) + 1e-5)
        for r0 in range(0, D, RP):
            st(hT, r0, RP, T(b), (ld(xT_s, r0, RP, T(b)).astype(F32) - mean) * rstd)
    def epi(which, b, r):
        if which == 0:
            for r0 in range(0, D, RP): st(pq, r0, RP, T(b), _phi(r[r0:r0+RP]))
        elif which == 1:
            for r0 in range(0, D, RP):
                k = _phi(r[r0:r0+RP])
                st(pk, r0, RP, T(b), k)
                if b == 0: zb_s[r0:r0+RP, :] = k
                else: zb_s[r0:r0+RP, :] = zb_s[r0:r0+RP, :] + k
        else:
            for r0 in range(0, D, RP): st(vT, r0, RP, T(b), r[r0:r0+RP])
    def G(which, b):
        epi(which, b, jnp.dot(ld(wqkvT, which*D, D, slice(None)), ld(xT_s, 0, D, T(b)), preferred_element_type=F32))
    def GO(which, b):
        cs = pl.ds(pl.multiple_of(sm[b], 128), 128)
        ro = pl.multiple_of(sm[4 + which], 256)
        lhs = pltpu.bitcast(wqkvT[pl.ds(ro, D // 2), :], BF)
        epi(which, b, jnp.dot(lhs, ld(xT_s, 0, D, cs), preferred_element_type=F32))
    def GT(which, b):
        r = lax.dot_general(ld(wqkv_ref, 0, D, slice(which*D, (which+1)*D)), ld(x_ref, b*128, 128, slice(None)),
                            (((0,), (1,)), ((), ())), preferred_element_type=F32)
        epi(which, b, r)
    def GW():
        gwb_s[...] = jnp.broadcast_to(gw_ref[...].astype(F32).reshape(1, D), (128, D)).T
    def Z():
        zb_s[...] = jnp.broadcast_to(jnp.sum(zb_s[...], axis=1, keepdims=True), (D, 128))
    def KV(gi):
        ri = lax.broadcasted_iota(jnp.int32, (128, 128), 0) // DH
        ci = lax.broadcasted_iota(jnp.int32, (128, 128), 1) // DH
        kv = lax.dot_general(ld(pk, gi*128, 128, slice(None)), ld(vT, gi*128, 128, slice(None)), NT, preferred_element_type=F32)
        st(kv_s, 0, 128, T(gi), jnp.where(ri == ci, kv, 0.0))
    def M(gi):
        r = lax.dot_general(ld(woT, 0, D, T(gi)), ld(kv_s, 0, 128, T(gi)), NT, preferred_element_type=F32)
        for r0 in range(0, D, RP): st(MT, r0, RP, T(gi), r[r0:r0+RP])
    done = set()
    def need(*deps):
        for d in deps: assert d in done, 'schedule dependency violated: %s' % d
    def run_seq(seq):
        for tok in seq.split():
            op, args = tok[0], tok[1:]
            assert tok not in done, tok
            if tok == 'GW': GW()
            elif tok == 'Z':
                need(*['G1.%d' % b for b in range(16)]); Z()
            elif op in 'TQG':
                w, b = map(int, args.split('.'))
                if op != 'T': need('X%d' % b, *['W%d' % (4*w + j) for j in range(4)])
                {'T': GT, 'Q': GO, 'G': G}[op](w, b)
                tok = 'G' + args
            elif op == 'W': W(int(args))
            elif op == 'O': WO(int(args))
            elif op == 'X': need('GW'); X(int(args))
            elif op == 'L': need('X' + args); L(int(args))
            elif op == 'K':
                need(*['G%d.%d' % (w, b) for w in (1, 2) for b in range(16)]); KV(int(args))
            elif op == 'M': need('K' + args, *['O%d' % j for j in range(4)]); M(int(args))
            else: raise ValueError(tok)
            done.add(tok)
    SA = ('T0.0 GW W0 W1 X0 X1 W2 W3 G0.1 X2 X3 G0.2')
    SB = ('Q0.3 W4 W5 W6 W7 G1.0 W8 W9 L0 G1.1 W10 W11 G1.2 L1 G1.3 G2.0 L2 G2.1 L3 G2.2')
    NQ = 2
    sc = ['X4 %s2.3 X5' % ('Q')]
    for b in range(4, 16):
        sc.append('G1.%d' % b)
        if b + 2 < 16: sc.append('X%d' % (b + 2))
        else: sc.append('O%d O%d' % (2*(b-14), 2*(b-14)+1))
        sc.append('G2.%d L%d' % (b, b))
        if b < 16 - NQ: sc.append('G0.%d' % b)
    dq = ['G0.%d' % b for b in range(16 - NQ, 16)]
    tail = ('K0 K1 Z K2 K3 q M0 M1 q M2 M3 q q')
    qi = 0
    for t in tail.split():
        if t == 'q':
            if qi < len(dq): sc.append(dq[qi]); qi += 1
        else: sc.append(t)
    sc += dq[qi:]
    SCs = (' '.join(sc))
    cx[0].wait(); cw[0].wait(); cgw.wait()
    run_seq(SA)
    cw[1].wait(); cw[2].wait()
    run_seq(SB)
    for c in range(1, nx): cx[c].wait()
    cwo.wait()
    run_seq(SCs)
    need(*(['L%d' % b for b in range(16)] + ['G0.%d' % b for b in range(16)] + ['M%d' % g for g in range(4)] + ['Z']))
    cw1.wait(); cb1.wait(); cb2.wait()
    b1_s[...] = b1_ref[...].astype(F32).reshape(1, F)
    b2_s[...] = b2_ref[...].astype(F32).reshape(1, S)

    def p2_chunk(f0, fc):
        fs = pl.ds(f0, fc)
        u = jnp.dot(pltpu.bitcast(hT[...], BF), pltpu.bitcast(w1_ref[:, fs], BF), preferred_element_type=F32)
        b1 = b1_s[:, fs]
        for r0 in range(0, D, RP): st(gu, r0, RP, fs, _gelu(u[r0:r0+RP] + b1))
    def PQ(s0):
        cs = pl.ds(s0, 128)
        for h0 in range(0, H, PH):
            r0, nr = h0 * DH, PH * DH
            t = ld(pq, r0, nr, cs).astype(F32)
            den = jnp.sum((t * zb_s[r0:r0+nr, :]).reshape(PH, DH, 128), axis=1, keepdims=True) + 1e-6
            st(pq, r0, nr, cs, (t.reshape(PH, DH, 128) * (1.0 / den)).reshape(nr, 128))
    C1 = F // N2
    NB1 = 16 // N2
    def b2_(i, c):
        base = pl.multiple_of(i * C1, 128)
        tb = pl.multiple_of(i * NB1 * 128, 128)
        nf = C1 // FC
        k = 0
        for j in range(nf):
            p2_chunk(base + j * FC, FC)
            while k < (NB1 * (j + 1) + nf - 2) // (nf - 1) and k < NB1:
                PQ(tb + k * 128); k += 1
        return c
    lax.fori_loop(0, N2, b2_, 0)
    cw2.wait()

    def p3_compute(s0, out_fn):
        sl = pl.ds(s0, OC)
        y = jnp.dot(pltpu.bitcast(gu[...], BF), pltpu.bitcast(w2_ref[:, sl], BF), preferred_element_type=F32)
        a = jnp.dot(pltpu.bitcast(MT[...], BF), pltpu.bitcast(pq[:, sl], BF), preferred_element_type=F32)
        g = g_s[0:1, sl]; b2 = b2_s[:, sl]
        g1 = 1.0 - g
        for r0 in range(0, D, RP):
            out_fn(r0, (g * a[r0:r0+RP] + g1 * (y[r0:r0+RP] + b2)).astype(BF))
    T3 = S // N3
    NS = T3 // OC
    def out_copy(r0, k):
        r0 = pl.multiple_of(r0 // 2, OC // 2)
        return pltpu.make_async_copy(o_ref.at[pl.ds(r0, OC // 2), :], oh.at[pl.ds(r0, OC // 2), :], sems.at[13 + k])
    def o_finish(r0, src):
        r0 = pl.multiple_of(r0 // 2, OC // 2)
        for c in range(4):
            o_ref[pl.ds(r0, OC // 2), T(c)] = pltpu.bitcast(ld(src, c*128, 128, slice(None)).T, U32)
    oT_s[NS - 1] = jnp.zeros((D // 2, OC), U32)
    def b3_(i, c):
        base = pl.multiple_of(i * T3, T3)
        FP = 0
        if FP == 0: o_finish(jnp.where(i == 0, S, base - OC), oT_s.at[NS - 1])
        for j in range(NS):
            buf = oT_s.at[j]
            if j == NS - 1 and FP == 2: o_finish(jnp.where(i == 0, S, base - OC), oT_s.at[NS - 1])
            p3_compute(base + j * OC, lambda r0, v: st(buf, r0, RP, slice(None), v))
            if j == 0 and FP == 1: o_finish(jnp.where(i == 0, S, base - OC), oT_s.at[NS - 1])
            if j < NS - 1: o_finish(base + j * OC, buf)
        @pl.when(i > 0)
        def _():
            out_copy(base - OC, i * NS - 1).start()
        for j in range(NS - 1):
            out_copy(base + j * OC, i * NS + j).start()
        return c
    lax.fori_loop(0, N3, b3_, 0)
    o_finish(S - OC, oT_s.at[NS - 1])
    out_copy(S - OC, N3 * NS - 1).start()
    for k in range(N3 * NS):
        out_copy(k * OC, k).wait()

@jax.jit
def pallas_gated_mix__linear_attn_block__mixer_token_mlp__prompt_kernel(A_x, A_wqkv, A_wo, B_x, B_w1, B_b1, B_w2, B_b2, gate_w):
    x = A_x.reshape(S, D)
    anyspec = pl.BlockSpec(memory_space=pl.ANY)
    P = lambda r, c: pltpu.VMEM((r // 2, c), U32)
    out = pl.pallas_call(
        kernel,
        out_shape=jax.ShapeDtypeStruct((S, D), BF),
        in_specs=[anyspec]*8, out_specs=anyspec,
        scratch_shapes=[
            P(S, D), P(D, 3*D), P(D, D), P(S, F), pltpu.VMEM((F,), BF),
            P(F, S), pltpu.VMEM((S,), BF), pltpu.VMEM((D,), BF), P(S + OC, D),
            P(3*D, D), P(D, D), P(D, S), P(D, S),
            P(D, S), P(D, S), P(D, S),
            P(D, F), P(D, D), pltpu.VMEM((2, S), F32),
            pltpu.VMEM((1, F), F32), pltpu.VMEM((1, S), F32), pltpu.VMEM((D, 128), F32), pltpu.VMEM((D, 128), F32),
            pltpu.VMEM((S // N3 // OC, D // 2, OC), U32), P(128, D),
            pltpu.SMEM((8,), jnp.int32),
            pltpu.SemaphoreType.DMA((40,)),
        ],
        compiler_params=pltpu.CompilerParams(vmem_limit_bytes=100*1024*1024),
    )(x, A_wqkv, A_wo, B_w1, B_b1, B_w2, B_b2, gate_w)
    return out.reshape(1, S, D)
```

```python
import numpy as np
import jax
import jax.numpy as jnp
from jax import lax
import jax.experimental.pallas as pl
import jax.experimental.pallas.tpu as pltpu

S, D, F, H, DH = 2048, 512, 1792, 32, 16
BF, F32, U32 = jnp.bfloat16, jnp.float32, jnp.uint32
NT = (((1,), (1,)), ((), ()))

N2 = 2
N3 = 4
OC = 256
PAD = 64

BATCHES = (
    ('xa', ('x0-128', 'w0-128')), ('xb', ('x128-256', 'w128-256')),
    ('xc', ('x256-384', 'w256-384')), ('xd', ('x384-512', 'w384-512')),
    ('wk', ('w512-1024', 'gw')), ('wv', ('w1024-1536',)), ('x1', ('x512-1024',)),
    ('x2', ('x1024-2048', 'wo')), ('w1', ('b1', 'b2', 'w1')), ('w2', ('w2',)),
)

PHASE1 = (
    'w:xa X0 W0 u0 w:xb X1 W1 u1 r1 w:xc X2 W2 u2 r2 w:xd X3 W3 u3 '
    'w:wk GW W4 W5 W6 W7 r3 Q1.0 L0 Q1.1 pw w:wv W8 W9 L1 Q1.2 W10 W11 Q1.3 L2 Q2.0 '
    'px w:x1 X4 X5 Q2.1 L3 Q2.2 Q2.3 '
    'G0.4 G1.4 X6 G2.4 L4 px w:x2 '
    + ' '.join('G0.%d G1.%d X%d G2.%d L%d' % (b, b, b + 2, b, b) for b in range(5, 14))
    + ' G1.14 O0 O1 G2.14 L14 G1.15 O2 O3 G2.15 L15 '
    'K0 K1 Z K2 K3 G0.14 G0.15 M0 M1 M2 M3 w:w1 BS'
)


def _phi(t):
    return jnp.where(t > 0, t + 1.0, jnp.exp(t)) + 1e-6


def _gelu(u):
    c = float(np.sqrt(2.0 / np.pi))
    return 0.5 * u * (1.0 + jnp.tanh(c * (u + 0.044715 * (u * u * u))))


def ld(ref, r0, nr, cs):
    return pltpu.bitcast(ref[pl.ds(r0 // 2, nr // 2), cs], BF)


def st(ref, r0, nr, cs, val):
    ref[pl.ds(r0 // 2, nr // 2), cs] = pltpu.bitcast(val.astype(BF), U32)


def colsum8(v):
    return jnp.sum(v.reshape(v.shape[0] // 8, 8, 128), axis=0)


def T(b):
    return slice(b * 128, (b + 1) * 128)


def kernel(x_hbm, wqkv_hbm, wo_hbm, w1_hbm, b1_hbm, w2_hbm, b2_hbm, gw_hbm, o_hbm,
           x_ref, wqkv_ref, wo_ref, w1_ref, b1_ref, w2_ref, b2_ref, gw_ref, o_ref,
           wqkvT, woT, xT_s, hT, pq, pk, vT, gu, MT, g_s, b1_s, b2_s, zb_s, gwb_s,
           oT_s, kv_s, sm, sems, zsem):
    xh, wqh, woh, w1h, w2h = (r.bitcast(U32) for r in (x_hbm, wqkv_hbm, wo_hbm, w1_hbm, w2_hbm))

    batches = {}
    for k, (name, items) in enumerate(BATCHES):
        lst = []
        for it in items:
            if it == 'wo':
                c = pltpu.make_async_copy(woh, wo_ref, sems.at[k])
            elif it == 'w1':
                c = pltpu.make_async_copy(w1h, w1_ref, sems.at[k])
            elif it == 'w2':
                c = pltpu.make_async_copy(w2h, w2_ref, sems.at[k])
            elif it == 'gw':
                c = pltpu.make_async_copy(gw_hbm, gw_ref, sems.at[k])
            elif it == 'b1':
                c = pltpu.make_async_copy(b1_hbm, b1_ref, sems.at[k])
            elif it == 'b2':
                c = pltpu.make_async_copy(b2_hbm, b2_ref, sems.at[k])
            else:
                lo, hi = (int(v) for v in it[1:].split('-'))
                if it[0] == 'x':
                    c = pltpu.make_async_copy(xh.at[lo // 2:hi // 2, :], x_ref.at[lo // 2:hi // 2, :], sems.at[k])
                else:
                    c = pltpu.make_async_copy(wqh.at[:, lo:hi], wqkv_ref.at[0:D // 2, lo:hi], sems.at[k])
            lst.append(c)
        batches[name] = lst
    for name, _ in BATCHES:
        for c in batches[name]:
            c.start()

    def wait(name):
        for c in batches[name]:
            c.wait()

    for b in range(16):
        sm[16 + b] = b * 128
    for b in range(12):
        sm[40 + b] = b * 64
    sm[7] = S // 2
    sm[8] = D // 2
    sm[9] = D // 2
    zero = pl.semaphore_read(zsem)

    def W(j):
        st(wqkvT, j * 128, 128, slice(None), ld(wqkv_ref, 0, D, T(j)).T)

    def WO(j):
        st(woT, j * 128, 128, slice(None), ld(wo_ref, 0, D, T(j)).T)

    def X(b):
        st(xT_s, 0, D, T(b), ld(x_ref, b * 128, 128, slice(None)).T)

    def L(b):
        cs, rp = T(b), 256
        s8 = g8 = v8 = None
        for r0 in range(0, D, rp):
            xf = ld(xT_s, r0, rp, cs).astype(F32)
            p = colsum8(xf)
            s8 = p if s8 is None else s8 + p
            p = colsum8(xf * gwb_s[r0:r0 + rp, :])
            g8 = p if g8 is None else g8 + p
        mean = jnp.sum(s8, axis=0, keepdims=True) * (1.0 / D)
        g_s[0:1, cs] = jax.nn.sigmoid(jnp.sum(g8, axis=0, keepdims=True))
        for r0 in range(0, D, rp):
            xc = ld(xT_s, r0, rp, cs).astype(F32) - mean
            p = colsum8(xc * xc)
            v8 = p if v8 is None else v8 + p
        rstd = lax.rsqrt(jnp.sum(v8, axis=0, keepdims=True) * (1.0 / D) + 1e-5)
        for r0 in range(0, D, rp):
            st(hT, r0, rp, cs, (ld(xT_s, r0, rp, cs).astype(F32) - mean) * rstd)

    last, npin = {}, {}

    def pin(ref, k):
        j = npin.get(k, 0)
        npin[k] = j + 1
        ref[pl.ds(pl.multiple_of(sm[k] + zero + 8 * (j // 4), 8), 8), T(j % 4)] = last['v']

    def epi(which, b, r):
        last['v'] = pltpu.bitcast(r[0:8, :], U32)
        if which == 0:
            st(pq, 0, D, T(b), _phi(r))
        elif which == 1:
            k = _phi(r)
            st(pk, 0, D, T(b), k)
            if b == 0:
                zb_s[...] = k
            else:
                zb_s[...] = zb_s[...] + k
        else:
            st(vT, 0, D, T(b), r)

    def lhs_o(k0, nr):
        return pltpu.bitcast(wqkvT[pl.ds(pl.multiple_of(sm[40 + k0 // 128], 64), nr // 2), :], BF)

    def rhs_o(b0, nc):
        return ld(xT_s, 0, D, pl.ds(pl.multiple_of(sm[16 + b0], 128), nc))

    def G(which, b):
        epi(which, b, jnp.dot(ld(wqkvT, which * D, D, slice(None)), ld(xT_s, 0, D, T(b)),
                              preferred_element_type=F32))

    def Q(which, b):
        epi(which, b, jnp.dot(lhs_o(which * D, D), rhs_o(b, 128), preferred_element_type=F32))

    def TU(k):
        r = jnp.dot(lhs_o(0, 128 * (k + 1)), rhs_o(k, 128), preferred_element_type=F32)
        last['v'] = pltpu.bitcast(r[0:8, :], U32)
        st(pq, 0, 128 * (k + 1), T(k), _phi(r))

    def TR(k):
        r = jnp.dot(lhs_o(128 * k, 128), rhs_o(0, 128 * k), preferred_element_type=F32)
        last['v'] = pltpu.bitcast(r[0:8, 0:128], U32)
        st(pq, 128 * k, 128, slice(0, 128 * k), _phi(r))

    def GW():
        gwb_s[...] = jnp.broadcast_to(gw_ref[...].astype(F32).reshape(1, D), (128, D)).T

    def Z():
        zb_s[...] = jnp.broadcast_to(jnp.sum(zb_s[...], axis=1, keepdims=True), (D, 128))

    def KV(gi):
        ri = lax.broadcasted_iota(jnp.int32, (128, 128), 0) // DH
        ci = lax.broadcasted_iota(jnp.int32, (128, 128), 1) // DH
        kv = lax.dot_general(ld(pk, gi * 128, 128, slice(None)), ld(vT, gi * 128, 128, slice(None)),
                             NT, preferred_element_type=F32)
        st(kv_s, 0, 128, T(gi), jnp.where(ri == ci, kv, 0.0))

    def M(gi):
        st(MT, 0, D, T(gi), lax.dot_general(ld(woT, 0, D, T(gi)), ld(kv_s, 0, 128, T(gi)),
                                            NT, preferred_element_type=F32))

    def BS():
        b1_s[...] = b1_ref[...].astype(F32).reshape(1, F)
        b2_s[...] = b2_ref[...].astype(F32).reshape(1, S)

    done = set()

    def need(*deps):
        for d in deps:
            assert d in done, 'phase-1 order violates a dependency: %s' % d

    for tok in PHASE1.split():
        op, args = tok[0], tok[1:]
        if tok.startswith('w:'):
            wait(tok[2:])
            continue
        if tok == 'px':
            pin(x_ref, 7)
            continue
        if tok == 'pw':
            pin(wqkv_ref, 8)
            continue
        assert tok not in done, tok
        if tok == 'GW':
            GW()
        elif tok == 'BS':
            BS()
        elif tok == 'Z':
            need(*['G1.%d' % b for b in range(16)])
            Z()
        elif op in 'QG':
            w, b = (int(v) for v in args.split('.'))
            need('X%d' % b, *['W%d' % (4 * w + j) for j in range(4)])
            (Q if op == 'Q' else G)(w, b)
            tok = 'G' + args
        elif op == 'u':
            k = int(args)
            need('X%d' % k, *['W%d' % j for j in range(k + 1)])
            TU(k)
        elif op == 'r':
            k = int(args)
            need('W%d' % k, *['X%d' % j for j in range(k)])
            TR(k)
            if k == 3:
                need('u0', 'u1', 'u2', 'u3', 'r1', 'r2')
                done.update('G0.%d' % b for b in range(4))
        elif op == 'W':
            W(int(args))
        elif op == 'O':
            WO(int(args))
        elif op == 'X':
            X(int(args))
        elif op == 'L':
            need('X' + args, 'GW')
            L(int(args))
        elif op == 'K':
            need(*['G%d.%d' % (w, b) for w in (1, 2) for b in range(16)])
            KV(int(args))
        elif op == 'M':
            need('K' + args, *['O%d' % j for j in range(4)])
            M(int(args))
        else:
            raise ValueError(tok)
        done.add(tok)
    need('BS', 'Z', *(['L%d' % b for b in range(16)] + ['G0.%d' % b for b in range(16)]
                      + ['M%d' % g for g in range(4)]))

    def p2_chunk(f0):
        fs = pl.ds(f0, 128)
        u = jnp.dot(pltpu.bitcast(hT[...], BF), pltpu.bitcast(w1_ref[:, fs], BF),
                    preferred_element_type=F32)
        st(gu, 0, D, fs, _gelu(u + b1_s[:, fs]))

    def PQ(s0):
        cs = pl.ds(s0, 128)
        for h in range(H):
            r0 = h * DH
            t = ld(pq, r0, DH, cs).astype(F32)
            den = jnp.sum((t * zb_s[r0:r0 + DH, :]).reshape(1, DH, 128), axis=1, keepdims=True) + 1e-6
            st(pq, r0, DH, cs, (t.reshape(1, DH, 128) * (1.0 / den)).reshape(DH, 128))

    C1, NB1 = F // N2, 16 // N2
    nf = C1 // 128

    def body2(i, c):
        base = pl.multiple_of(i * C1, 128)
        tb = pl.multiple_of(i * NB1 * 128, 128)
        k = 0
        for j in range(nf):
            p2_chunk(base + j * 128)
            while k < (NB1 * (j + 1) + nf - 2) // (nf - 1) and k < NB1:
                PQ(tb + k * 128)
                k += 1
        return c

    lax.fori_loop(0, N2, body2, 0)
    wait('w2')

    T3 = S // N3
    NS = T3 // OC

    def out_copy(r0):
        r0 = pl.multiple_of(r0, OC)
        return pltpu.make_async_copy(o_ref.at[pl.ds(r0, OC), :], o_hbm.at[pl.ds(r0, OC), :], sems.at[0])

    def body3(i, c):
        base = pl.multiple_of(i * T3, T3)
        for j in range(NS):
            s0 = base + j * OC
            sl = pl.ds(s0, OC)
            y = jnp.dot(pltpu.bitcast(gu[...], BF), pltpu.bitcast(w2_ref[:, sl], BF),
                        preferred_element_type=F32)
            a = jnp.dot(pltpu.bitcast(MT[...], BF), pltpu.bitcast(pq[:, sl], BF),
                        preferred_element_type=F32)
            g = g_s[0:1, sl]
            st(oT_s.at[j], 0, D, slice(None), g * a + (1.0 - g) * (y + b2_s[:, sl]))
            r0 = pl.multiple_of(s0, OC)
            for cb in range(4):
                o_ref[pl.ds(r0, OC), T(cb)] = ld(oT_s.at[j], cb * 128, 128, slice(None)).T
            out_copy(s0).start()
        return c

    lax.fori_loop(0, N3, body3, 0)
    for k in range(N3 * NS):
        out_copy(k * OC).wait()


@jax.jit
def pallas_gated_mix__linear_attn_block__mixer_token_mlp__prompt_kernel(
    A_x: jax.Array,
    A_wqkv: jax.Array,
    A_wo: jax.Array,
    B_x: jax.Array,
    B_w1: jax.Array,
    B_b1: jax.Array,
    B_w2: jax.Array,
    B_b2: jax.Array,
    gate_w: jax.Array,
):
    del B_x
    anyspec = pl.BlockSpec(memory_space=pl.ANY)

    def P(r, c):
        return pltpu.VMEM((r // 2, c), U32)

    out = pl.pallas_call(
        kernel,
        out_shape=jax.ShapeDtypeStruct((S, D), BF),
        in_specs=[anyspec] * 8,
        out_specs=anyspec,
        scratch_shapes=[
            P(S + PAD, D), P(D + PAD, 3 * D), P(D, D), P(S, F), pltpu.VMEM((F,), BF),
            P(F, S), pltpu.VMEM((S,), BF), pltpu.VMEM((D,), BF), pltpu.VMEM((S, D), BF),
            P(3 * D, D), P(D, D), P(D, S), P(D, S), P(D, S), P(D, S), P(D, S), P(D, F), P(D, D),
            pltpu.VMEM((2, S), F32), pltpu.VMEM((1, F), F32), pltpu.VMEM((1, S), F32),
            pltpu.VMEM((D, 128), F32), pltpu.VMEM((D, 128), F32),
            pltpu.VMEM((S // N3 // OC, D // 2, OC), U32), P(128, D),
            pltpu.SMEM((64,), jnp.int32),
            pltpu.SemaphoreType.DMA((len(BATCHES),)),
            pltpu.SemaphoreType.REGULAR,
        ],
        compiler_params=pltpu.CompilerParams(
            vmem_limit_bytes=100 * 1024 * 1024,
            flags={'XLA_TPU_RESCHEDULE_DMA_DONES': True},
        ),
    )(A_x.reshape(S, D), A_wqkv, A_wo, B_w1, B_b1, B_w2, B_b2, gate_w)
    return out.reshape(1, S, D)
```

```python
import numpy as np
import jax
import jax.numpy as jnp
from jax import lax
import jax.experimental.pallas as pl
import jax.experimental.pallas.tpu as pltpu

S, D, F, H, DH = 2048, 512, 1792, 32, 16
BF, F32, U32 = jnp.bfloat16, jnp.float32, jnp.uint32
NT = (((1,), (1,)), ((), ()))

N2 = 2
N3 = 4
OC = 256
PAD = 16

BATCHES = (
    ('xa', ('x0-128', 'w0-128')), ('xb', ('x128-256', 'w128-256')),
    ('xc', ('x256-384', 'w256-384')), ('xd', ('x384-512', 'w384-512')),
    ('wk', ('w512-1024', 'gw')), ('wv', ('w1024-1536',)), ('x1', ('x512-1024',)),
    ('x2', ('x1024-2048', 'wo')), ('w1', ('b1', 'b2', 'w1')), ('w2', ('w2',)),
)

PHASE1 = (
    'w:xa X0 W0 u0 w:xb X1 W1 u1 r1 w:xc X2 W2 u2 r2 w:xd X3 W3 u3 '
    'w:wk GW W4 W5 W6 W7 r3 Q1.0 L0 Q1.1 pw w:wv W8 W9 L1 Q1.2 W10 W11 Q1.3 L2 Q2.0 '
    'px w:x1 X4 X5 Q2.1 L3 Q2.2 Q2.3 '
    'G0.4 G1.4 X6 G2.4 L4 px w:x2 '
    + ' '.join('G0.%d G1.%d X%d G2.%d L%d' % (b, b, b + 2, b, b) for b in range(5, 14))
    + ' G1.14 O0 O1 G2.14 L14 G1.15 O2 O3 G2.15 L15 '
    'K0 K1 Z K2 K3 G0.14 G0.15 M0 M1 M2 M3 w:w1 BS'
)


def _phi(t):
    return jnp.where(t > 0, t + 1.0, jnp.exp(t)) + 1e-6


def _gelu(u):
    c = float(np.sqrt(2.0 / np.pi))
    return 0.5 * u * (1.0 + jnp.tanh(c * (u + 0.044715 * (u * u * u))))


def ld(ref, r0, nr, cs):
    return pltpu.bitcast(ref[pl.ds(r0 // 2, nr // 2), cs], BF)


def st(ref, r0, nr, cs, val):
    ref[pl.ds(r0 // 2, nr // 2), cs] = pltpu.bitcast(val.astype(BF), U32)


def colsum8(v):
    return jnp.sum(v.reshape(v.shape[0] // 8, 8, 128), axis=0)


def T(b):
    return slice(b * 128, (b + 1) * 128)


def kernel(x_hbm, wqkv_hbm, wo_hbm, w1_hbm, b1_hbm, w2_hbm, b2_hbm, gw_hbm, o_hbm,
           x_ref, wqkv_ref, wo_ref, w1_ref, b1_ref, w2_ref, b2_ref, gw_ref, o_ref,
           wqkvT, woT, xT_s, hT, pq, pk, vT, gu, MT, g_s, b1_s, b2_s, zb_s, gwb_s,
           oT_s, kv_s, sm, sems):
    xh, wqh, woh, w1h, w2h = (r.bitcast(U32) for r in (x_hbm, wqkv_hbm, wo_hbm, w1_hbm, w2_hbm))

    batches = {}
    for k, (name, items) in enumerate(BATCHES):
        lst = []
        for it in items:
            if it == 'wo':
                c = pltpu.make_async_copy(woh, wo_ref, sems.at[k])
            elif it == 'w1':
                c = pltpu.make_async_copy(w1h, w1_ref, sems.at[k])
            elif it == 'w2':
                c = pltpu.make_async_copy(w2h, w2_ref, sems.at[k])
            elif it == 'gw':
                c = pltpu.make_async_copy(gw_hbm, gw_ref, sems.at[k])
            elif it == 'b1':
                c = pltpu.make_async_copy(b1_hbm, b1_ref, sems.at[k])
            elif it == 'b2':
                c = pltpu.make_async_copy(b2_hbm, b2_ref, sems.at[k])
            else:
                lo, hi = (int(v) for v in it[1:].split('-'))
                if it[0] == 'x':
                    c = pltpu.make_async_copy(xh.at[lo // 2:hi // 2, :], x_ref.at[lo // 2:hi // 2, :], sems.at[k])
                else:
                    c = pltpu.make_async_copy(wqh.at[:, lo:hi], wqkv_ref.at[0:D // 2, lo:hi], sems.at[k])
            lst.append(c)
        batches[name] = lst
    for name, _ in BATCHES:
        for c in batches[name]:
            c.start()

    def wait(name):
        for c in batches[name]:
            c.wait()

    for b in range(16):
        sm[16 + b] = b * 128
    for b in range(12):
        sm[40 + b] = b * 64

    def W(j):
        st(wqkvT, j * 128, 128, slice(None), ld(wqkv_ref, 0, D, T(j)).T)

    def WO(j):
        st(woT, j * 128, 128, slice(None), ld(wo_ref, 0, D, T(j)).T)

    def X(b):
        st(xT_s, 0, D, T(b), ld(x_ref, b * 128, 128, slice(None)).T)

    def L(b):
        cs, rp = T(b), 256
        s8 = g8 = v8 = None
        for r0 in range(0, D, rp):
            xf = ld(xT_s, r0, rp, cs).astype(F32)
            p = colsum8(xf)
            s8 = p if s8 is None else s8 + p
            p = colsum8(xf * gwb_s[r0:r0 + rp, :])
            g8 = p if g8 is None else g8 + p
        mean = jnp.sum(s8, axis=0, keepdims=True) * (1.0 / D)
        g_s[0:1, cs] = jax.nn.sigmoid(jnp.sum(g8, axis=0, keepdims=True))
        for r0 in range(0, D, rp):
            xc = ld(xT_s, r0, rp, cs).astype(F32) - mean
            p = colsum8(xc * xc)
            v8 = p if v8 is None else v8 + p
        rstd = lax.rsqrt(jnp.sum(v8, axis=0, keepdims=True) * (1.0 / D) + 1e-5)
        for r0 in range(0, D, rp):
            st(hT, r0, rp, cs, (ld(xT_s, r0, rp, cs).astype(F32) - mean) * rstd)

    last, npin = {}, {}

    def pin(ref, row0):
        j = npin.get(row0, 0)
        npin[row0] = j + 1
        ref[row0 + 8 * (j // 4):row0 + 8 * (j // 4) + 8, T(j % 4)] = last['v']

    def epi(which, b, r):
        last['v'] = pltpu.bitcast(r[0:8, :], U32)
        if which == 0:
            st(pq, 0, D, T(b), _phi(r))
        elif which == 1:
            k = _phi(r)
            st(pk, 0, D, T(b), k)
            if b == 0:
                zb_s[...] = k
            else:
                zb_s[...] = zb_s[...] + k
        else:
            st(vT, 0, D, T(b), r)

    def lhs_o(k0, nr):
        return pltpu.bitcast(wqkvT[pl.ds(pl.multiple_of(sm[40 + k0 // 128], 64), nr // 2), :], BF)

    def rhs_o(b0, nc):
        return ld(xT_s, 0, D, pl.ds(pl.multiple_of(sm[16 + b0], 128), nc))

    def G(which, b):
        epi(which, b, jnp.dot(ld(wqkvT, which * D, D, slice(None)), ld(xT_s, 0, D, T(b)),
                              preferred_element_type=F32))

    def Q(which, b):
        epi(which, b, jnp.dot(lhs_o(which * D, D), rhs_o(b, 128), preferred_element_type=F32))

    def TU(k):
        r = jnp.dot(lhs_o(0, 128 * (k + 1)), rhs_o(k, 128), preferred_element_type=F32)
        last['v'] = pltpu.bitcast(r[0:8, :], U32)
        st(pq, 0, 128 * (k + 1), T(k), _phi(r))

    def TR(k):
        r = jnp.dot(lhs_o(128 * k, 128), rhs_o(0, 128 * k), preferred_element_type=F32)
        last['v'] = pltpu.bitcast(r[0:8, 0:128], U32)
        st(pq, 128 * k, 128, slice(0, 128 * k), _phi(r))

    def GW():
        gwb_s[...] = jnp.broadcast_to(gw_ref[...].astype(F32).reshape(1, D), (128, D)).T

    def Z():
        zb_s[...] = jnp.broadcast_to(jnp.sum(zb_s[...], axis=1, keepdims=True), (D, 128))

    def KV(gi):
        ri = lax.broadcasted_iota(jnp.int32, (128, 128), 0) // DH
        ci = lax.broadcasted_iota(jnp.int32, (128, 128), 1) // DH
        kv = lax.dot_general(ld(pk, gi * 128, 128, slice(None)), ld(vT, gi * 128, 128, slice(None)),
                             NT, preferred_element_type=F32)
        st(kv_s, 0, 128, T(gi), jnp.where(ri == ci, kv, 0.0))

    def M(gi):
        st(MT, 0, D, T(gi), lax.dot_general(ld(woT, 0, D, T(gi)), ld(kv_s, 0, 128, T(gi)),
                                            NT, preferred_element_type=F32))

    def BS():
        b1_s[...] = b1_ref[...].astype(F32).reshape(1, F)
        b2_s[...] = b2_ref[...].astype(F32).reshape(1, S)

    done = set()

    def need(*deps):
        for d in deps:
            assert d in done, 'phase-1 order violates a dependency: %s' % d

    for tok in PHASE1.split():
        op, args = tok[0], tok[1:]
        if tok.startswith('w:'):
            wait(tok[2:])
            continue
        if tok == 'px':
            pin(x_ref, S // 2)
            continue
        if tok == 'pw':
            pin(wqkv_ref, D // 2)
            continue
        assert tok not in done, tok
        if tok == 'GW':
            GW()
        elif tok == 'BS':
            BS()
        elif tok == 'Z':
            need(*['G1.%d' % b for b in range(16)])
            Z()
        elif op in 'QG':
            w, b = (int(v) for v in args.split('.'))
            need('X%d' % b, *['W%d' % (4 * w + j) for j in range(4)])
            (Q if op == 'Q' else G)(w, b)
            tok = 'G' + args
        elif op == 'u':
            k = int(args)
            need('X%d' % k, *['W%d' % j for j in range(k + 1)])
            TU(k)
        elif op == 'r':
            k = int(args)
            need('W%d' % k, *['X%d' % j for j in range(k)])
            TR(k)
            if k == 3:
                need('u0', 'u1', 'u2', 'u3', 'r1', 'r2')
                done.update('G0.%d' % b for b in range(4))
        elif op == 'W':
            W(int(args))
        elif op == 'O':
            WO(int(args))
        elif op == 'X':
            X(int(args))
        elif op == 'L':
            need('X' + args, 'GW')
            L(int(args))
        elif op == 'K':
            need(*['G%d.%d' % (w, b) for w in (1, 2) for b in range(16)])
            KV(int(args))
        elif op == 'M':
            need('K' + args, *['O%d' % j for j in range(4)])
            M(int(args))
        else:
            raise ValueError(tok)
        done.add(tok)
    need('BS', 'Z', *(['L%d' % b for b in range(16)] + ['G0.%d' % b for b in range(16)]
                      + ['M%d' % g for g in range(4)]))

    def p2_chunk(f0):
        fs = pl.ds(f0, 128)
        u = jnp.dot(pltpu.bitcast(hT[...], BF), pltpu.bitcast(w1_ref[:, fs], BF),
                    preferred_element_type=F32)
        st(gu, 0, D, fs, _gelu(u + b1_s[:, fs]))

    def PQ(s0):
        cs = pl.ds(s0, 128)
        for h in range(H):
            r0 = h * DH
            t = ld(pq, r0, DH, cs).astype(F32)
            den = jnp.sum((t * zb_s[r0:r0 + DH, :]).reshape(1, DH, 128), axis=1, keepdims=True) + 1e-6
            st(pq, r0, DH, cs, (t.reshape(1, DH, 128) * (1.0 / den)).reshape(DH, 128))

    C1, NB1 = F // N2, 16 // N2
    nf = C1 // 128

    def body2(i, c):
        base = pl.multiple_of(i * C1, 128)
        tb = pl.multiple_of(i * NB1 * 128, 128)
        k = 0
        for j in range(nf):
            p2_chunk(base + j * 128)
            while k < (NB1 * (j + 1) + nf - 2) // (nf - 1) and k < NB1:
                PQ(tb + k * 128)
                k += 1
        return c

    lax.fori_loop(0, N2, body2, 0)
    wait('w2')

    T3 = S // N3
    NS = T3 // OC

    def out_copy(r0):
        r0 = pl.multiple_of(r0, OC)
        return pltpu.make_async_copy(o_ref.at[pl.ds(r0, OC), :], o_hbm.at[pl.ds(r0, OC), :], sems.at[0])

    def body3(i, c):
        base = pl.multiple_of(i * T3, T3)
        for j in range(NS):
            s0 = base + j * OC
            sl = pl.ds(s0, OC)
            y = jnp.dot(pltpu.bitcast(gu[...], BF), pltpu.bitcast(w2_ref[:, sl], BF),
                        preferred_element_type=F32)
            a = jnp.dot(pltpu.bitcast(MT[...], BF), pltpu.bitcast(pq[:, sl], BF),
                        preferred_element_type=F32)
            g = g_s[0:1, sl]
            st(oT_s.at[j], 0, D, slice(None), g * a + (1.0 - g) * (y + b2_s[:, sl]))
            r0 = pl.multiple_of(s0, OC)
            for cb in range(4):
                o_ref[pl.ds(r0, OC), T(cb)] = ld(oT_s.at[j], cb * 128, 128, slice(None)).T
            out_copy(s0).start()
        return c

    lax.fori_loop(0, N3, body3, 0)
    for k in range(N3 * NS):
        out_copy(k * OC).wait()


@jax.jit
def pallas_gated_mix__linear_attn_block__mixer_token_mlp__prompt_kernel(
    A_x: jax.Array,
    A_wqkv: jax.Array,
    A_wo: jax.Array,
    B_x: jax.Array,
    B_w1: jax.Array,
    B_b1: jax.Array,
    B_w2: jax.Array,
    B_b2: jax.Array,
    gate_w: jax.Array,
):
    del B_x
    anyspec = pl.BlockSpec(memory_space=pl.ANY)

    def P(r, c):
        return pltpu.VMEM((r // 2, c), U32)

    out = pl.pallas_call(
        kernel,
        out_shape=jax.ShapeDtypeStruct((S, D), BF),
        in_specs=[anyspec] * 8,
        out_specs=anyspec,
        scratch_shapes=[
            P(S + PAD, D), P(D + PAD, 3 * D), P(D, D), P(S, F), pltpu.VMEM((F,), BF),
            P(F, S), pltpu.VMEM((S,), BF), pltpu.VMEM((D,), BF), pltpu.VMEM((S, D), BF),
            P(3 * D, D), P(D, D), P(D, S), P(D, S), P(D, S), P(D, S), P(D, S), P(D, F), P(D, D),
            pltpu.VMEM((2, S), F32), pltpu.VMEM((1, F), F32), pltpu.VMEM((1, S), F32),
            pltpu.VMEM((D, 128), F32), pltpu.VMEM((D, 128), F32),
            pltpu.VMEM((S // N3 // OC, D // 2, OC), U32), P(128, D),
            pltpu.SMEM((64,), jnp.int32),
            pltpu.SemaphoreType.DMA((len(BATCHES),)),
        ],
        compiler_params=pltpu.CompilerParams(
            vmem_limit_bytes=100 * 1024 * 1024,
            flags={'XLA_TPU_RESCHEDULE_DMA_DONES': True},
        ),
    )(A_x.reshape(S, D), A_wqkv, A_wo, B_w1, B_b1, B_w2, B_b2, gate_w)
    return out.reshape(1, S, D)
```

```python
import numpy as np
import jax
import jax.numpy as jnp
from jax import lax
import jax.experimental.pallas as pl
import jax.experimental.pallas.tpu as pltpu

S, D, F, H, DH = 2048, 512, 1792, 32, 16
BF, F32, U32 = jnp.bfloat16, jnp.float32, jnp.uint32
NT = (((1,), (1,)), ((), ()))

N2 = 2
N3 = 4
OC = 128
PAD = 16

BATCHES = (
    ('xa', ('x0-128', 'w0-128')), ('xb', ('x128-256', 'w128-256')),
    ('xc', ('x256-384', 'w256-384')), ('xd', ('x384-512', 'w384-512')),
    ('wk', ('w512-1024', 'gw')), ('wv', ('w1024-1536',)), ('x1', ('x512-1024',)),
    ('x2', ('x1024-2048', 'wo')), ('w1', ('b1', 'b2', 'w1')), ('w2', ('w2',)),
)

PHASE1 = (
    'w:xa X0 W0 u0 w:xb X1 W1 u1 r1 w:xc X2 W2 u2 r2 w:xd X3 W3 u3 '
    'w:wk GW W4 W5 W6 W7 r3 Q1.0 L0 Q1.1 pw w:wv W8 W9 L1 Q1.2 W10 W11 Q1.3 L2 Q2.0 '
    'px w:x1 X4 X5 Q2.1 L3 Q2.2 Q2.3 '
    'G0.4 G1.4 X6 G2.4 L4 px w:x2 '
    + ' '.join('G0.%d G1.%d X%d G2.%d L%d' % (b, b, b + 2, b, b) for b in range(5, 14))
    + ' G1.14 O0 O1 G2.14 L14 G1.15 O2 O3 G2.15 L15 '
    'K0 K1 Z K2 K3 G0.14 G0.15 M0 M1 M2 M3 w:w1 BS'
)


def _phi(t):
    return jnp.where(t > 0, t + 1.0, jnp.exp(t)) + 1e-6


def _gelu(u):
    c = float(np.sqrt(2.0 / np.pi))
    return 0.5 * u * (1.0 + jnp.tanh(c * (u + 0.044715 * (u * u * u))))


def ld(ref, r0, nr, cs):
    return pltpu.bitcast(ref[pl.ds(r0 // 2, nr // 2), cs], BF)


def st(ref, r0, nr, cs, val):
    ref[pl.ds(r0 // 2, nr // 2), cs] = pltpu.bitcast(val.astype(BF), U32)


def colsum8(v):
    return jnp.sum(v.reshape(v.shape[0] // 8, 8, 128), axis=0)


def T(b):
    return slice(b * 128, (b + 1) * 128)


def kernel(x_hbm, wqkv_hbm, wo_hbm, w1_hbm, b1_hbm, w2_hbm, b2_hbm, gw_hbm, o_hbm,
           x_ref, wqkv_ref, wo_ref, w1_ref, b1_ref, w2_ref, b2_ref, gw_ref, o_ref,
           wqkvT, woT, xT_s, hT, pq, pk, vT, gu, MT, g_s, b1_s, b2_s, zb_s, gwb_s,
           oT_s, kv_s, sm, sems):
    xh, wqh, woh, w1h, w2h = (r.bitcast(U32) for r in (x_hbm, wqkv_hbm, wo_hbm, w1_hbm, w2_hbm))

    batches = {}
    for k, (name, items) in enumerate(BATCHES):
        lst = []
        for it in items:
            if it == 'wo':
                c = pltpu.make_async_copy(woh, wo_ref, sems.at[k])
            elif it == 'w1':
                c = pltpu.make_async_copy(w1h, w1_ref, sems.at[k])
            elif it == 'w2':
                c = pltpu.make_async_copy(w2h, w2_ref, sems.at[k])
            elif it == 'gw':
                c = pltpu.make_async_copy(gw_hbm, gw_ref, sems.at[k])
            elif it == 'b1':
                c = pltpu.make_async_copy(b1_hbm, b1_ref, sems.at[k])
            elif it == 'b2':
                c = pltpu.make_async_copy(b2_hbm, b2_ref, sems.at[k])
            else:
                lo, hi = (int(v) for v in it[1:].split('-'))
                if it[0] == 'x':
                    c = pltpu.make_async_copy(xh.at[lo // 2:hi // 2, :], x_ref.at[lo // 2:hi // 2, :], sems.at[k])
                else:
                    c = pltpu.make_async_copy(wqh.at[:, lo:hi], wqkv_ref.at[0:D // 2, lo:hi], sems.at[k])
            lst.append(c)
        batches[name] = lst
    for name, _ in BATCHES:
        for c in batches[name]:
            c.start()

    def wait(name):
        for c in batches[name]:
            c.wait()

    for b in range(16):
        sm[16 + b] = b * 128
    for b in range(12):
        sm[40 + b] = b * 64

    def W(j):
        st(wqkvT, j * 128, 128, slice(None), ld(wqkv_ref, 0, D, T(j)).T)

    def WO(j):
        st(woT, j * 128, 128, slice(None), ld(wo_ref, 0, D, T(j)).T)

    def X(b):
        st(xT_s, 0, D, T(b), ld(x_ref, b * 128, 128, slice(None)).T)

    def L(b):
        cs, rp = T(b), 256
        s8 = g8 = v8 = None
        for r0 in range(0, D, rp):
            xf = ld(xT_s, r0, rp, cs).astype(F32)
            p = colsum8(xf)
            s8 = p if s8 is None else s8 + p
            p = colsum8(xf * gwb_s[r0:r0 + rp, :])
            g8 = p if g8 is None else g8 + p
        mean = jnp.sum(s8, axis=0, keepdims=True) * (1.0 / D)
        g_s[0:1, cs] = jax.nn.sigmoid(jnp.sum(g8, axis=0, keepdims=True))
        for r0 in range(0, D, rp):
            xc = ld(xT_s, r0, rp, cs).astype(F32) - mean
            p = colsum8(xc * xc)
            v8 = p if v8 is None else v8 + p
        rstd = lax.rsqrt(jnp.sum(v8, axis=0, keepdims=True) * (1.0 / D) + 1e-5)
        for r0 in range(0, D, rp):
            st(hT, r0, rp, cs, (ld(xT_s, r0, rp, cs).astype(F32) - mean) * rstd)

    last, npin = {}, {}

    def pin(ref, row0):
        j = npin.get(row0, 0)
        npin[row0] = j + 1
        ref[row0 + 8 * (j // 4):row0 + 8 * (j // 4) + 8, T(j % 4)] = last['v']

    def epi(which, b, r):
        last['v'] = pltpu.bitcast(r[0:8, :], U32)
        if which == 0:
            st(pq, 0, D, T(b), _phi(r))
        elif which == 1:
            k = _phi(r)
            st(pk, 0, D, T(b), k)
            if b == 0:
                zb_s[...] = k
            else:
                zb_s[...] = zb_s[...] + k
        else:
            st(vT, 0, D, T(b), r)

    def lhs_o(k0, nr):
        return pltpu.bitcast(wqkvT[pl.ds(pl.multiple_of(sm[40 + k0 // 128], 64), nr // 2), :], BF)

    def rhs_o(b0, nc):
        return ld(xT_s, 0, D, pl.ds(pl.multiple_of(sm[16 + b0], 128), nc))

    def G(which, b):
        epi(which, b, jnp.dot(ld(wqkvT, which * D, D, slice(None)), ld(xT_s, 0, D, T(b)),
                              preferred_element_type=F32))

    def Q(which, b):
        epi(which, b, jnp.dot(lhs_o(which * D, D), rhs_o(b, 128), preferred_element_type=F32))

    def TU(k):
        r = jnp.dot(lhs_o(0, 128 * (k + 1)), rhs_o(k, 128), preferred_element_type=F32)
        last['v'] = pltpu.bitcast(r[0:8, :], U32)
        st(pq, 0, 128 * (k + 1), T(k), _phi(r))

    def TR(k):
        r = jnp.dot(lhs_o(128 * k, 128), rhs_o(0, 128 * k), preferred_element_type=F32)
        last['v'] = pltpu.bitcast(r[0:8, 0:128], U32)
        st(pq, 128 * k, 128, slice(0, 128 * k), _phi(r))

    def GW():
        gwb_s[...] = jnp.broadcast_to(gw_ref[...].astype(F32).reshape(1, D), (128, D)).T

    def Z():
        zb_s[...] = jnp.broadcast_to(jnp.sum(zb_s[...], axis=1, keepdims=True), (D, 128))

    def KV(gi):
        ri = lax.broadcasted_iota(jnp.int32, (128, 128), 0) // DH
        ci = lax.broadcasted_iota(jnp.int32, (128, 128), 1) // DH
        kv = lax.dot_general(ld(pk, gi * 128, 128, slice(None)), ld(vT, gi * 128, 128, slice(None)),
                             NT, preferred_element_type=F32)
        st(kv_s, 0, 128, T(gi), jnp.where(ri == ci, kv, 0.0))

    def M(gi):
        st(MT, 0, D, T(gi), lax.dot_general(ld(woT, 0, D, T(gi)), ld(kv_s, 0, 128, T(gi)),
                                            NT, preferred_element_type=F32))

    def BS():
        b1_s[...] = b1_ref[...].astype(F32).reshape(1, F)
        b2_s[...] = b2_ref[...].astype(F32).reshape(1, S)

    done = set()

    def need(*deps):
        for d in deps:
            assert d in done, 'phase-1 order violates a dependency: %s' % d

    for tok in PHASE1.split():
        op, args = tok[0], tok[1:]
        if tok.startswith('w:'):
            wait(tok[2:])
            continue
        if tok == 'px':
            pin(x_ref, S // 2)
            continue
        if tok == 'pw':
            pin(wqkv_ref, D // 2)
            continue
        assert tok not in done, tok
        if tok == 'GW':
            GW()
        elif tok == 'BS':
            BS()
        elif tok == 'Z':
            need(*['G1.%d' % b for b in range(16)])
            Z()
        elif op in 'QG':
            w, b = (int(v) for v in args.split('.'))
            need('X%d' % b, *['W%d' % (4 * w + j) for j in range(4)])
            (Q if op == 'Q' else G)(w, b)
            tok = 'G' + args
        elif op == 'u':
            k = int(args)
            need('X%d' % k, *['W%d' % j for j in range(k + 1)])
            TU(k)
        elif op == 'r':
            k = int(args)
            need('W%d' % k, *['X%d' % j for j in range(k)])
            TR(k)
            if k == 3:
                need('u0', 'u1', 'u2', 'u3', 'r1', 'r2')
                done.update('G0.%d' % b for b in range(4))
        elif op == 'W':
            W(int(args))
        elif op == 'O':
            WO(int(args))
        elif op == 'X':
            X(int(args))
        elif op == 'L':
            need('X' + args, 'GW')
            L(int(args))
        elif op == 'K':
            need(*['G%d.%d' % (w, b) for w in (1, 2) for b in range(16)])
            KV(int(args))
        elif op == 'M':
            need('K' + args, *['O%d' % j for j in range(4)])
            M(int(args))
        else:
            raise ValueError(tok)
        done.add(tok)
    need('BS', 'Z', *(['L%d' % b for b in range(16)] + ['G0.%d' % b for b in range(16)]
                      + ['M%d' % g for g in range(4)]))

    def p2_chunk(f0):
        fs = pl.ds(f0, 128)
        u = jnp.dot(pltpu.bitcast(hT[...], BF), pltpu.bitcast(w1_ref[:, fs], BF),
                    preferred_element_type=F32)
        st(gu, 0, D, fs, _gelu(u + b1_s[:, fs]))

    def PQ(s0):
        cs = pl.ds(s0, 128)
        for h in range(H):
            r0 = h * DH
            t = ld(pq, r0, DH, cs).astype(F32)
            den = jnp.sum((t * zb_s[r0:r0 + DH, :]).reshape(1, DH, 128), axis=1, keepdims=True) + 1e-6
            st(pq, r0, DH, cs, (t.reshape(1, DH, 128) * (1.0 / den)).reshape(DH, 128))

    C1, NB1 = F // N2, 16 // N2
    nf = C1 // 128

    def body2(i, c):
        base = pl.multiple_of(i * C1, 128)
        tb = pl.multiple_of(i * NB1 * 128, 128)
        k = 0
        for j in range(nf):
            p2_chunk(base + j * 128)
            while k < (NB1 * (j + 1) + nf - 2) // (nf - 1) and k < NB1:
                PQ(tb + k * 128)
                k += 1
        return c

    lax.fori_loop(0, N2, body2, 0)
    wait('w2')

    T3 = S // N3
    NP = T3 // OC
    zero = pl.program_id(0)
    A0 = S + OC

    def out_copy(r0):
        r0 = pl.multiple_of(r0, OC)
        return pltpu.make_async_copy(o_ref.at[pl.ds(r0, OC), :], o_hbm.at[pl.ds(r0, OC), :], sems.at[0])

    def finish(r0, j):
        r0 = pl.multiple_of(r0, OC)
        for cb in range(4):
            o_ref[pl.ds(r0, OC), T(cb)] = ld(oT_s.at[j], cb * 128, 128, slice(None)).T

    def anchor_store(j, slot):
        o_ref[A0:A0 + 16, T(slot)] = pltpu.bitcast(oT_s[j, 0:8, :], BF)

    def anchored(w2v, slot):
        dummy = pltpu.bitcast(o_ref[pl.ds(pl.multiple_of(A0 + zero, 16), 16), T(slot)], U32)
        m = dummy & jnp.full((8, 128), zero, jnp.int32).astype(U32)
        k0 = 6 * 64
        return jnp.concatenate([w2v[0:k0], w2v[k0:k0 + 8] | m, w2v[k0 + 8:]], axis=0)

    oT_s[NP - 1] = jnp.zeros((D // 2, OC), U32)

    def body3(i, c):
        base = pl.multiple_of(i * T3, T3)
        finish(jnp.where(i == 0, S, base - OC), NP - 1)

        @pl.when(i > 0)
        def _():
            out_copy(base - OC).start()

        anchor_store(NP - 1, NP - 1)
        for j in range(NP):
            s0 = base + j * OC
            sl = pl.ds(s0, OC)
            w2v = anchored(w2_ref[:, sl], (j - 1) % NP)
            y = jnp.dot(pltpu.bitcast(gu[...], BF), pltpu.bitcast(w2v, BF),
                        preferred_element_type=F32)
            a = jnp.dot(pltpu.bitcast(MT[...], BF), pltpu.bitcast(pq[:, sl], BF),
                        preferred_element_type=F32)
            g = g_s[0:1, sl]
            st(oT_s.at[j], 0, D, slice(None), g * a + (1.0 - g) * (y + b2_s[:, sl]))
            if j < NP - 1:
                finish(s0, j)
                out_copy(s0).start()
                anchor_store(j, j)
        return c

    lax.fori_loop(0, N3, body3, 0)
    finish(S - OC, NP - 1)
    out_copy(S - OC).start()
    for k in range(S // OC):
        out_copy(k * OC).wait()


@jax.jit
def pallas_gated_mix__linear_attn_block__mixer_token_mlp__prompt_kernel(
    A_x: jax.Array,
    A_wqkv: jax.Array,
    A_wo: jax.Array,
    B_x: jax.Array,
    B_w1: jax.Array,
    B_b1: jax.Array,
    B_w2: jax.Array,
    B_b2: jax.Array,
    gate_w: jax.Array,
):
    del B_x
    anyspec = pl.BlockSpec(memory_space=pl.ANY)

    def P(r, c):
        return pltpu.VMEM((r // 2, c), U32)

    out = pl.pallas_call(
        kernel,
        out_shape=jax.ShapeDtypeStruct((S, D), BF),
        grid=(1,),
        in_specs=[anyspec] * 8,
        out_specs=anyspec,
        scratch_shapes=[
            P(S + PAD, D), P(D + PAD, 3 * D), P(D, D), P(S, F), pltpu.VMEM((F,), BF),
            P(F, S), pltpu.VMEM((S,), BF), pltpu.VMEM((D,), BF), pltpu.VMEM((S + OC + 16, D), BF),
            P(3 * D, D), P(D, D), P(D, S), P(D, S), P(D, S), P(D, S), P(D, S), P(D, F), P(D, D),
            pltpu.VMEM((2, S), F32), pltpu.VMEM((1, F), F32), pltpu.VMEM((1, S), F32),
            pltpu.VMEM((D, 128), F32), pltpu.VMEM((D, 128), F32),
            pltpu.VMEM((S // N3 // OC, D // 2, OC), U32), P(128, D),
            pltpu.SMEM((64,), jnp.int32),
            pltpu.SemaphoreType.DMA((len(BATCHES),)),
        ],
        compiler_params=pltpu.CompilerParams(
            vmem_limit_bytes=100 * 1024 * 1024,
            flags={'XLA_TPU_RESCHEDULE_DMA_DONES': True},
        ),
    )(A_x.reshape(S, D), A_wqkv, A_wo, B_w1, B_b1, B_w2, B_b2, gate_w)
    return out.reshape(1, S, D)
```

```python
import numpy as np
import jax
import jax.numpy as jnp
from jax import lax
import jax.experimental.pallas as pl
import jax.experimental.pallas.tpu as pltpu

S, D, F, H, DH = 2048, 512, 1792, 32, 16
BF, F32, U32 = jnp.bfloat16, jnp.float32, jnp.uint32
NT = (((1,), (1,)), ((), ()))

N2 = 2
N3 = 4
OC = 128
PAD = 16

BATCHES = (
    ('xa', ('x0-128', 'w0-128')), ('xb', ('x128-256', 'w128-256')),
    ('xc', ('x256-384', 'w256-384')), ('xd', ('x384-512', 'w384-512')),
    ('wk', ('w512-1024', 'gw')), ('wv', ('w1024-1536',)), ('x1', ('x512-1024',)),
    ('x2', ('x1024-2048', 'wo')), ('w1', ('b1', 'b2', 'w1')), ('w2', ('w2',)),
)

PHASE1 = (
    'w:xa X0 W0 u0 w:xb X1 W1 u1 r1 w:xc X2 W2 u2 r2 w:xd X3 W3 u3 '
    'w:wk GW W4 W5 W6 W7 r3 Q1.0 L0 Q1.1 pw w:wv W8 W9 L1 Q1.2 W10 W11 Q1.3 L2 Q2.0 '
    'px w:x1 X4 X5 Q2.1 L3 Q2.2 Q2.3 '
    'G0.4 G1.4 X6 G2.4 L4 px w:x2 '
    + ' '.join('G0.%d G1.%d X%d G2.%d L%d' % (b, b, b + 2, b, b) for b in range(5, 14))
    + ' G1.14 O0 O1 G2.14 L14 G1.15 O2 O3 G2.15 L15 '
    'K0 K1 Z K2 K3 G0.14 G0.15 M0 M1 M2 M3 p1 w:w1 BS'
)


def _phi(t):
    return jnp.where(t > 0, t + 1.0, jnp.exp(t)) + 1e-6


def _gelu(u):
    c = float(np.sqrt(2.0 / np.pi))
    return 0.5 * u * (1.0 + jnp.tanh(c * (u + 0.044715 * (u * u * u))))


def ld(ref, r0, nr, cs):
    return pltpu.bitcast(ref[pl.ds(r0 // 2, nr // 2), cs], BF)


def st(ref, r0, nr, cs, val):
    ref[pl.ds(r0 // 2, nr // 2), cs] = pltpu.bitcast(val.astype(BF), U32)


def colsum8(v):
    return jnp.sum(v.reshape(v.shape[0] // 8, 8, 128), axis=0)


def T(b):
    return slice(b * 128, (b + 1) * 128)


def kernel(x_hbm, wqkv_hbm, wo_hbm, w1_hbm, b1_hbm, w2_hbm, b2_hbm, gw_hbm, o_hbm,
           x_ref, wqkv_ref, wo_ref, w1_ref, b1_ref, w2_ref, b2_ref, gw_ref, o_ref,
           wqkvT, woT, xT_s, hT, pq, pk, vT, gu, MT, g_s, b1_s, b2_s, zb_s, gwb_s,
           oT_s, kv_s, sm, sems):

    batches = {}
    for k, (name, items) in enumerate(BATCHES):
        lst = []
        for it in items:
            if it == 'wo':
                c = pltpu.make_async_copy(wo_hbm, wo_ref, sems.at[k])
            elif it == 'w1':
                c = pltpu.make_async_copy(w1_hbm, w1_ref.at[0:S, :], sems.at[k])
            elif it == 'w2':
                c = pltpu.make_async_copy(w2_hbm, w2_ref, sems.at[k])
            elif it == 'gw':
                c = pltpu.make_async_copy(gw_hbm, gw_ref, sems.at[k])
            elif it == 'b1':
                c = pltpu.make_async_copy(b1_hbm, b1_ref, sems.at[k])
            elif it == 'b2':
                c = pltpu.make_async_copy(b2_hbm, b2_ref, sems.at[k])
            else:
                lo, hi = (int(v) for v in it[1:].split('-'))
                if it[0] == 'x':
                    c = pltpu.make_async_copy(x_hbm.at[lo:hi, :], x_ref.at[lo:hi, :], sems.at[k])
                else:
                    c = pltpu.make_async_copy(wqkv_hbm.at[:, lo:hi], wqkv_ref.at[0:D, lo:hi], sems.at[k])
            lst.append(c)
        batches[name] = lst
    for name, _ in BATCHES:
        for c in batches[name]:
            c.start()

    def wait(name):
        for c in batches[name]:
            c.wait()

    for b in range(16):
        sm[16 + b] = b * 128
    for b in range(12):
        sm[40 + b] = b * 64

    def W(j):
        st(wqkvT, j * 128, 128, slice(None), wqkv_ref[0:D, T(j)].T)

    def WO(j):
        st(woT, j * 128, 128, slice(None), wo_ref[:, T(j)].T)

    def X(b):
        st(xT_s, 0, D, T(b), x_ref[b * 128:(b + 1) * 128, :].T)

    def L(b):
        cs, rp = T(b), 256
        s8 = g8 = v8 = None
        for r0 in range(0, D, rp):
            xf = ld(xT_s, r0, rp, cs).astype(F32)
            p = colsum8(xf)
            s8 = p if s8 is None else s8 + p
            p = colsum8(xf * gwb_s[r0:r0 + rp, :])
            g8 = p if g8 is None else g8 + p
        mean = jnp.sum(s8, axis=0, keepdims=True) * (1.0 / D)
        g_s[0:1, cs] = jax.nn.sigmoid(jnp.sum(g8, axis=0, keepdims=True))
        for r0 in range(0, D, rp):
            xc = ld(xT_s, r0, rp, cs).astype(F32) - mean
            p = colsum8(xc * xc)
            v8 = p if v8 is None else v8 + p
        rstd = lax.rsqrt(jnp.sum(v8, axis=0, keepdims=True) * (1.0 / D) + 1e-5)
        for r0 in range(0, D, rp):
            st(hT, r0, rp, cs, (ld(xT_s, r0, rp, cs).astype(F32) - mean) * rstd)

    last, npin = {}, {}

    def pin(ref, row0):
        j = npin.get(row0, 0)
        npin[row0] = j + 1
        ref[row0 + 16 * (j // 4):row0 + 16 * (j // 4) + 16, T(j % 4)] = pltpu.bitcast(last['v'], BF)

    def epi(which, b, r):
        last['v'] = pltpu.bitcast(r[0:8, :], U32)
        if which == 0:
            st(pq, 0, D, T(b), _phi(r))
        elif which == 1:
            k = _phi(r)
            st(pk, 0, D, T(b), k)
            if b == 0:
                zb_s[...] = k
            else:
                zb_s[...] = zb_s[...] + k
        else:
            st(vT, 0, D, T(b), r)

    def lhs_o(k0, nr):
        return pltpu.bitcast(wqkvT[pl.ds(pl.multiple_of(sm[40 + k0 // 128], 64), nr // 2), :], BF)

    def rhs_o(b0, nc):
        return ld(xT_s, 0, D, pl.ds(pl.multiple_of(sm[16 + b0], 128), nc))

    def G(which, b):
        epi(which, b, jnp.dot(ld(wqkvT, which * D, D, slice(None)), ld(xT_s, 0, D, T(b)),
                              preferred_element_type=F32))

    def Q(which, b):
        epi(which, b, jnp.dot(lhs_o(which * D, D), rhs_o(b, 128), preferred_element_type=F32))

    def TU(k):
        r = jnp.dot(lhs_o(0, 128 * (k + 1)), rhs_o(k, 128), preferred_element_type=F32)
        last['v'] = pltpu.bitcast(r[0:8, :], U32)
        st(pq, 0, 128 * (k + 1), T(k), _phi(r))

    def TR(k):
        r = jnp.dot(lhs_o(128 * k, 128), rhs_o(0, 128 * k), preferred_element_type=F32)
        last['v'] = pltpu.bitcast(r[0:8, 0:128], U32)
        st(pq, 128 * k, 128, slice(0, 128 * k), _phi(r))

    def GW():
        gwb_s[...] = jnp.broadcast_to(gw_ref[...].astype(F32).reshape(1, D), (128, D)).T

    def Z():
        zb_s[...] = jnp.broadcast_to(jnp.sum(zb_s[...], axis=1, keepdims=True), (D, 128))

    def KV(gi):
        ri = lax.broadcasted_iota(jnp.int32, (128, 128), 0) // DH
        ci = lax.broadcasted_iota(jnp.int32, (128, 128), 1) // DH
        kv = lax.dot_general(ld(pk, gi * 128, 128, slice(None)), ld(vT, gi * 128, 128, slice(None)),
                             NT, preferred_element_type=F32)
        st(kv_s, 0, 128, T(gi), jnp.where(ri == ci, kv, 0.0))

    def M(gi):
        st(MT, 0, D, T(gi), lax.dot_general(ld(woT, 0, D, T(gi)), ld(kv_s, 0, 128, T(gi)),
                                            NT, preferred_element_type=F32))

    def BS():
        b1_s[...] = b1_ref[...].astype(F32).reshape(1, F)
        b2_s[...] = b2_ref[...].astype(F32).reshape(1, S)

    done = set()

    def need(*deps):
        for d in deps:
            assert d in done, 'phase-1 order violates a dependency: %s' % d

    for tok in PHASE1.split():
        op, args = tok[0], tok[1:]
        if tok.startswith('w:'):
            wait(tok[2:])
            continue
        if tok == 'px':
            pin(x_ref, S)
            continue
        if tok == 'p1':
            pin(w1_ref, S)
            continue
        if tok == 'pw':
            pin(wqkv_ref, D)
            continue
        assert tok not in done, tok
        if tok == 'GW':
            GW()
        elif tok == 'BS':
            BS()
        elif tok == 'Z':
            need(*['G1.%d' % b for b in range(16)])
            Z()
        elif op in 'QG':
            w, b = (int(v) for v in args.split('.'))
            need('X%d' % b, *['W%d' % (4 * w + j) for j in range(4)])
            (Q if op == 'Q' else G)(w, b)
            tok = 'G' + args
        elif op == 'u':
            k = int(args)
            need('X%d' % k, *['W%d' % j for j in range(k + 1)])
            TU(k)
        elif op == 'r':
            k = int(args)
            need('W%d' % k, *['X%d' % j for j in range(k)])
            TR(k)
            if k == 3:
                need('u0', 'u1', 'u2', 'u3', 'r1', 'r2')
                done.update('G0.%d' % b for b in range(4))
        elif op == 'W':
            W(int(args))
        elif op == 'O':
            WO(int(args))
        elif op == 'X':
            X(int(args))
        elif op == 'L':
            need('X' + args, 'GW')
            L(int(args))
        elif op == 'K':
            need(*['G%d.%d' % (w, b) for w in (1, 2) for b in range(16)])
            KV(int(args))
        elif op == 'M':
            need('K' + args, *['O%d' % j for j in range(4)])
            M(int(args))
        else:
            raise ValueError(tok)
        done.add(tok)
    need('BS', 'Z', *(['L%d' % b for b in range(16)] + ['G0.%d' % b for b in range(16)]
                      + ['M%d' % g for g in range(4)]))

    def p2_chunk(f0):
        fs = pl.ds(f0, 128)
        u = jnp.dot(pltpu.bitcast(hT[...], BF), w1_ref[0:S, fs],
                    preferred_element_type=F32)
        st(gu, 0, D, fs, _gelu(u + b1_s[:, fs]))

    def PQ(s0):
        cs = pl.ds(s0, 128)
        for h in range(H):
            r0 = h * DH
            t = ld(pq, r0, DH, cs).astype(F32)
            den = jnp.sum((t * zb_s[r0:r0 + DH, :]).reshape(1, DH, 128), axis=1, keepdims=True) + 1e-6
            st(pq, r0, DH, cs, (t.reshape(1, DH, 128) * (1.0 / den)).reshape(DH, 128))

    C1, NB1 = F // N2, 16 // N2
    nf = C1 // 128

    def body2(i, c):
        base = pl.multiple_of(i * C1, 128)
        tb = pl.multiple_of(i * NB1 * 128, 128)
        k = 0
        for j in range(nf):
            p2_chunk(base + j * 128)
            while k < (NB1 * (j + 1) + nf - 2) // (nf - 1) and k < NB1:
                PQ(tb + k * 128)
                k += 1
        return c

    lax.fori_loop(0, N2, body2, 0)
    wait('w2')

    T3 = S // N3
    NP = T3 // OC
    zero = pl.program_id(0)
    A0 = S + OC

    def out_copy(r0):
        r0 = pl.multiple_of(r0, OC)
        return pltpu.make_async_copy(o_ref.at[pl.ds(r0, OC), :], o_hbm.at[pl.ds(r0, OC), :], sems.at[0])

    def finish(r0, j):
        r0 = pl.multiple_of(r0, OC)
        for cb in range(4):
            o_ref[pl.ds(r0, OC), T(cb)] = ld(oT_s.at[j], cb * 128, 128, slice(None)).T

    def anchor_store(j, slot):
        o_ref[A0:A0 + 16, T(slot)] = pltpu.bitcast(oT_s[j, 0:8, :], BF)

    def anchored(w2v, slot):
        dummy = pltpu.bitcast(o_ref[pl.ds(pl.multiple_of(A0 + zero, 16), 16), T(slot)], U32)
        m = dummy & jnp.full((8, 128), zero, jnp.int32).astype(U32)
        k0 = 6 * 64
        return jnp.concatenate([w2v[0:k0], w2v[k0:k0 + 8] | m, w2v[k0 + 8:]], axis=0)

    oT_s[NP - 1] = jnp.zeros((D // 2, OC), U32)

    def body3(i, c):
        base = pl.multiple_of(i * T3, T3)
        finish(jnp.where(i == 0, S, base - OC), NP - 1)

        @pl.when(i > 0)
        def _():
            out_copy(base - OC).start()

        anchor_store(NP - 1, NP - 1)
        for j in range(NP):
            s0 = base + j * OC
            sl = pl.ds(s0, OC)
            w2v = anchored(pltpu.bitcast(w2_ref[:, sl], U32), (j - 1) % NP)
            y = jnp.dot(pltpu.bitcast(gu[...], BF), pltpu.bitcast(w2v, BF),
                        preferred_element_type=F32)
            a = jnp.dot(pltpu.bitcast(MT[...], BF), pltpu.bitcast(pq[:, sl], BF),
                        preferred_element_type=F32)
            g = g_s[0:1, sl]
            st(oT_s.at[j], 0, D, slice(None), g * a + (1.0 - g) * (y + b2_s[:, sl]))
            if j < NP - 1:
                finish(s0, j)
                out_copy(s0).start()
                anchor_store(j, j)
        return c

    lax.fori_loop(0, N3, body3, 0)
    finish(S - OC, NP - 1)
    out_copy(S - OC).start()
    for k in range(S // OC):
        out_copy(k * OC).wait()


@jax.jit
def pallas_gated_mix__linear_attn_block__mixer_token_mlp__prompt_kernel(
    A_x: jax.Array,
    A_wqkv: jax.Array,
    A_wo: jax.Array,
    B_x: jax.Array,
    B_w1: jax.Array,
    B_b1: jax.Array,
    B_w2: jax.Array,
    B_b2: jax.Array,
    gate_w: jax.Array,
):
    del B_x
    anyspec = pl.BlockSpec(memory_space=pl.ANY)

    def P(r, c):
        return pltpu.VMEM((r // 2, c), U32)

    out = pl.pallas_call(
        kernel,
        out_shape=jax.ShapeDtypeStruct((S, D), BF),
        grid=(1,),
        in_specs=[anyspec] * 8,
        out_specs=anyspec,
        scratch_shapes=[
            pltpu.VMEM((S + PAD, D), BF), pltpu.VMEM((D + PAD, 3 * D), BF), pltpu.VMEM((D, D), BF),
            pltpu.VMEM((S + PAD, F), BF), pltpu.VMEM((F,), BF),
            pltpu.VMEM((F, S), BF), pltpu.VMEM((S,), BF), pltpu.VMEM((D,), BF), pltpu.VMEM((S + OC + 16, D), BF),
            P(3 * D, D), P(D, D), P(D, S), P(D, S), P(D, S), P(D, S), P(D, S), P(D, F), P(D, D),
            pltpu.VMEM((2, S), F32), pltpu.VMEM((1, F), F32), pltpu.VMEM((1, S), F32),
            pltpu.VMEM((D, 128), F32), pltpu.VMEM((D, 128), F32),
            pltpu.VMEM((S // N3 // OC, D // 2, OC), U32), P(128, D),
            pltpu.SMEM((64,), jnp.int32),
            pltpu.SemaphoreType.DMA((len(BATCHES),)),
        ],
        compiler_params=pltpu.CompilerParams(
            vmem_limit_bytes=100 * 1024 * 1024,
            flags={'XLA_TPU_RESCHEDULE_DMA_DONES': True},
        ),
    )(A_x.reshape(S, D), A_wqkv, A_wo, B_w1, B_b1, B_w2, B_b2, gate_w)
    return out.reshape(1, S, D)
```
